```python
import jax
import jax.numpy as jnp

def _softmax(x, axis=-1):
    return jax.nn.softmax(x, axis=axis)
def _gelu(x):
    return jax.nn.gelu(x, approximate=True)
def _silu(x):
    return jax.nn.silu(x)
def _sigmoid(x):
    return jax.nn.sigmoid(x)
def _layernorm(x, axis=-1, eps=1e-5):
    m = jnp.mean(x, axis=axis, keepdims=True)
    v = jnp.var(x, axis=axis, keepdims=True)
    return (x - m) / jnp.sqrt(v + eps)
def _scatter_add(tgt, idx, src, axis=0):
    return tgt.at[idx].add(src)
def _segment_sum(src, seg, n):
    return jax.ops.segment_sum(src, seg, n)
class _Rng:
    def __init__(self, key):
        self._k = key
    def _next(self):
        self._k, sub = jax.random.split(self._k)
        return sub
    def normal(self, shape):
        return jax.random.normal(self._next(), shape, dtype=jnp.bfloat16)
    def randint(self, lo, hi, shape):
        return jax.random.randint(self._next(), shape, lo, hi, dtype=jnp.int32)
    def uniform(self, shape, lo=0.0, hi=1.0):
        return jax.random.uniform(self._next(), shape, jnp.bfloat16, lo, hi)
    def permutation(self, n):
        return jax.random.permutation(self._next(), n)


kernel_name = 'gated_mix__compressed_kv_cla__sliding_block_cached__decode'

def setup_inputs():
    _rng = _Rng(jax.random.key(int.from_bytes(__import__("os").urandom(4), "little")))
    _w = (lambda a: (lambda t: t.astype(jnp.bfloat16) if jnp.issubdtype(t.dtype, jnp.floating) else t)(jnp.asarray(a)))
    def _A_setup():
        B, H, Sq, Sk, D, M = 8, 32, 1, 4096, 128, 512
        Dc = 4 * D
        return {
            "x": _w((lambda *s: _rng.normal(s) * 0.05)(B, Sq, M)),
            "c_kv": _w((lambda *s: _rng.normal(s) * 0.05)(B, Sk, Dc)),
            "w_q": _w((lambda *s: _rng.normal(s) * 0.05)(M, H, D) * (M ** -0.5)),
            "w_uk": _w((lambda *s: _rng.normal(s) * 0.05)(Dc, H, D) * (Dc ** -0.5)),
            "w_uv": _w((lambda *s: _rng.normal(s) * 0.05)(Dc, H, D) * (Dc ** -0.5)),
            "w_o": _w((lambda *s: _rng.normal(s) * 0.05)(H, D, M) * ((H * D) ** -0.5)),
        }
    _A_in = _A_setup()

    def _B_setup():
        B, Sq, D = 8, 1, 512
        Hq, Hkv, Sk, Dh = 32, 8, 4096, 128
        assert Hq % Hkv == 0, (Hq, Hkv)
        return {
            "x": _w((lambda *s: _rng.normal(s) * 0.05)(B, Sq, D)),
            "k_cache": _w((lambda *s: _rng.normal(s) * 0.05)(B, Hkv, Sk, Dh)),
            "v_cache": _w((lambda *s: _rng.normal(s) * 0.05)(B, Hkv, Sk, Dh)),
            "wq": _w((lambda *s: _rng.normal(s) * 0.05)(D, Hq * Dh) * (D ** -0.5)),
            "wo": _w((lambda *s: _rng.normal(s) * 0.05)(Hq * Dh, D) * ((Hq * Dh) ** -0.5)),
        }
    _B_in = _B_setup()

    return {
        "A_x": _A_in["x"],
        "A_c_kv": _A_in["c_kv"],
        "A_w_q": _A_in["w_q"],
        "A_w_uk": _A_in["w_uk"],
        "A_w_uv": _A_in["w_uv"],
        "A_w_o": _A_in["w_o"],
        "B_x": _B_in["x"],
        "B_k_cache": _B_in["k_cache"],
        "B_v_cache": _B_in["v_cache"],
        "B_wq": _B_in["wq"],
        "B_wo": _B_in["wo"],
        "gate_w": _w((lambda *s: _rng.normal(s) * 0.05)(512)),
    }

def reference(A_x, A_c_kv, A_w_q, A_w_uk, A_w_uv, A_w_o, B_x, B_k_cache, B_v_cache, B_wq, B_wo, gate_w):
    def _A_ref(x, c_kv, w_q, w_uk, w_uv, w_o):
        B, Sq, M = x.shape[0], x.shape[1], x.shape[2]
        Sk = c_kv.shape[1]
        H, D = w_q.shape[1], w_q.shape[2]
        q = jnp.einsum("bqm,mhd->bhqd", x, w_q)
        k = jnp.einsum("bkc,chd->bhkd", c_kv, w_uk)
        v = jnp.einsum("bkc,chd->bhkd", c_kv, w_uv)
        scores = jnp.einsum("bhqd,bhkd->bhqk", q, k) * (D ** -0.5)
        off = Sk - Sq
        qi = jnp.arange(Sq)[:, None]
        kj = jnp.arange(Sk)[None, :]
        cmask = kj <= (qi + off)
        scores = jnp.where(cmask[None, None], scores, -1e9)
        p = _softmax(scores, axis=-1)
        ctx = jnp.einsum("bhqk,bhkd->bhqd", p, v)
        return jnp.einsum("bhqd,hdm->bqm", ctx, w_o)

    def _B_ref(x, k_cache, v_cache, wq, wo):
        B, Sq, D = x.shape
        Hq, Dh = 32, 128
        Hkv, Sk = k_cache.shape[1], k_cache.shape[2]
        W = min(4096, max(256, Sk // 4))
        rep = Hq // Hkv
        q = (lambda x, *d: x.transpose(*d))((x @ wq).reshape(B, Sq, Hq, Dh), 0, 2, 1, 3)
        k = jnp.repeat(k_cache[:, :, Sk - W:, :], rep, axis=1)
        v = jnp.repeat(v_cache[:, :, Sk - W:, :], rep, axis=1)
        scores = jnp.einsum("bhqd,bhkd->bhqk", q, k) * (Dh ** -0.5)
        p = _softmax(scores, axis=-1)
        o = jnp.einsum("bhqk,bhkd->bhqd", p, v)
        return (lambda x, *d: x.transpose(*d))(o, 0, 2, 1, 3).reshape(B, Sq, Hq * Dh) @ wo

    x = A_x
    g = _sigmoid((x * gate_w).sum(-1, keepdims=True))
    a = _A_ref(x, A_c_kv, A_w_q, A_w_uk, A_w_uv, A_w_o)
    b = _B_ref(x, B_k_cache, B_v_cache, B_wq, B_wo)
    return g * a + (1 - g) * b
```

```python
import functools

import jax
import jax.numpy as jnp
import jax.experimental.pallas as pl
import jax.experimental.pallas.tpu as pltpu

_BF = jnp.bfloat16
_F32 = jnp.float32

_NT = (((1,), (1,)), ((), ()))


def _dot(a, b):
    return jnp.dot(a, b, preferred_element_type=_F32)


def _dot_nt(a, b):
    return jax.lax.dot_general(a, b, _NT, preferred_element_type=_F32)


def _head_pair(s_u32, hp, n_rows, n_pairs):
    v = s_u32[pl.ds(hp, n_rows, stride=n_pairs), :]
    lo = pltpu.unpack_elementwise(v, index=0, packed_dtype=_BF, unpacked_dtype=_F32)
    hi = pltpu.unpack_elementwise(v, index=1, packed_dtype=_BF, unpacked_dtype=_F32)
    return lo.astype(_BF), hi.astype(_BF)


def _kernel(x_ref, gw_ref, ckv_hbm, wq_hbm, wuk_hbm, wuv_hbm, wo_hbm, kc_hbm,
            vc_hbm, bq_hbm, bo_hbm, out_ref,
            s_wq, s_wuk, s_wuv, s_wo, s_bq, s_bo, s_ckv, s_k, s_v,
            s_q, s_qa, s_qb, s_cx, s_ob, s_sc, sems,
            *, B, H, D, M, C, Sk, Hkv, W, KB, mode):
    scale_a = float(D) ** -0.5
    scale_b = float(128) ** -0.5
    HP = H // 2
    rep = H // Hkv

    copies = {}

    def add(name, src, dst):
        copies[name] = pltpu.make_async_copy(src, dst, sems.at[len(copies)])

    add("wq", wq_hbm.bitcast(jnp.uint32), s_wq)
    add("wuk", wuk_hbm.bitcast(jnp.uint32), s_wuk)
    add("bq", bq_hbm, s_bq)
    for b in range(B):
        add(("ckv", b), ckv_hbm.at[b], s_ckv.at[b])
    add("wuv", wuv_hbm.bitcast(jnp.uint32), s_wuv)
    add("wo", wo_hbm, s_wo)
    for b in range(B):
        add(("k", b), kc_hbm.at[b, :, pl.ds(Sk - W, W), :], s_k.at[b])
        add(("v", b), vc_hbm.at[b, :, pl.ds(Sk - W, W), :], s_v.at[b])
    NBO = 4
    bo_rows = (H * D) // NBO
    for i in range(NBO):
        add(("bo", i), bo_hbm.at[pl.ds(i * bo_rows, bo_rows)],
            s_bo.at[pl.ds(i * bo_rows, bo_rows)])

    if mode != "compute":
        for c in copies.values():
            c.start()

    def wait(name):
        if mode != "compute":
            copies[name].wait()

    xb = x_ref[...]

    wait("wq")

    @pl.loop(0, HP)
    def _(hp):
        w0, w1 = _head_pair(s_wq, hp, M, HP)
        s_q[2 * hp] = _dot(xb, w0)
        s_q[2 * hp + 1] = _dot(xb, w1)

    wait("wuk")

    @pl.loop(0, HP)
    def _(hp):
        w0, w1 = _head_pair(s_wuk, hp, C, HP)
        for j, w in enumerate((w0, w1)):
            h = 2 * hp + j
            qa = _dot_nt(s_q[h].astype(_BF), w) * scale_a
            for ct in range(C // 128):
                s_qa[ct, pl.ds(pl.multiple_of(h * B, B), B), :] = qa[:, ct * 128:(ct + 1) * 128]

    wait("bq")
    qb_all = _dot(xb, s_bq[...]) * scale_b
    for h in range(H):
        s_qb[h * B:(h + 1) * B, :] = qb_all[:, h * 128:(h + 1) * 128]

    NKB = Sk // KB

    for b in range(B):
        wait(("ckv", b))
        q = jnp.concatenate(
            [s_qa[ct, pl.ds(b, H, stride=B), :] for ct in range(C // 128)],
            axis=1).astype(_BF)

        def score_body(kb, m):
            k0 = pl.multiple_of(kb * KB, KB)
            s = _dot_nt(q, s_ckv[b, pl.ds(k0, KB), :])
            s_sc[:, pl.ds(k0, KB)] = s
            return jnp.maximum(m, s)

        m = jax.lax.fori_loop(0, NKB, score_body,
                              jnp.full((H, KB), -jnp.inf, _F32), unroll=True)
        m = jnp.max(m, axis=1, keepdims=True)

        def pv_body(kb, carry):
            l, acc = carry
            k0 = pl.multiple_of(kb * KB, KB)
            p = jnp.exp(s_sc[:, pl.ds(k0, KB)] - m)
            acc = acc + _dot(p.astype(_BF), s_ckv[b, pl.ds(k0, KB), :])
            return l + p, acc

        l, acc = jax.lax.fori_loop(
            0, NKB, pv_body,
            (jnp.zeros((H, KB), _F32), jnp.zeros((H, C), _F32)), unroll=True)
        l = jnp.sum(l, axis=1, keepdims=True)
        cx = acc / l
        for ct in range(C // 128):
            s_cx[ct, b * H:(b + 1) * H, :] = cx[:, ct * 128:(ct + 1) * 128]

    wait("wuv")
    wait("wo")

    def proj_a(hp, acc):
        w0, w1 = _head_pair(s_wuv, hp, C, HP)
        for j, w in enumerate((w0, w1)):
            h = 2 * hp + j
            cxh = jnp.concatenate(
                [s_cx[ct, pl.ds(h, B, stride=H), :] for ct in range(C // 128)],
                axis=1).astype(_BF)
            ctx = _dot(cxh, w).astype(_BF)
            acc = acc + _dot(ctx, s_wo[pl.ds(pl.multiple_of(h * D, D), D), :])
        return acc

    out_a = jax.lax.fori_loop(0, HP, proj_a, jnp.zeros((B, M), _F32))

    G = 16 // rep
    grp = jax.lax.broadcasted_iota(jnp.int32, (16, W), 0) // rep
    grp_o = jax.lax.broadcasted_iota(jnp.int32, (16, 128), 0) // rep
    for b in range(B):
        wait(("k", b))
        qb = s_qb[pl.ds(b, H, stride=B), :].astype(_BF)
        ps = []
        for j in range(H // 16):
            q16 = qb[16 * j:16 * (j + 1)]
            s = None
            for i in range(G):
                si = _dot_nt(q16, s_k[b, G * j + i])
                s = si if s is None else jnp.where(grp == i, si, s)
            m = jnp.max(s, axis=1, keepdims=True)
            p = jnp.exp(s - m)
            l = jnp.sum(p, axis=1, keepdims=True)
            ps.append((p.astype(_BF), l))
        wait(("v", b))
        for j in range(H // 16):
            p, l = ps[j]
            o = None
            for i in range(G):
                oi = _dot(p, s_v[b, G * j + i])
                o = oi if o is None else jnp.where(grp_o == i, oi, o)
            s_ob[b * H + 16 * j:b * H + 16 * (j + 1), :] = o / l

    out_b = jnp.zeros((B, M), _F32)
    hs = H // NBO
    for i in range(NBO):
        wait(("bo", i))
        for h in range(i * hs, (i + 1) * hs):
            oh = s_ob[pl.ds(h, B, stride=H), :].astype(_BF)
            out_b = out_b + _dot(oh, s_bo[h * 128:(h + 1) * 128, :])

    xf = xb.astype(_F32)
    g = jax.nn.sigmoid(jnp.sum(xf * gw_ref[...].astype(_F32), axis=1, keepdims=True))
    out_ref[...] = (g * out_a + (1.0 - g) * out_b).astype(out_ref.dtype)


def _build(mode="full", KB=512):
    def fn(A_x, A_c_kv, A_w_q, A_w_uk, A_w_uv, A_w_o, B_x, B_k_cache, B_v_cache,
           B_wq, B_wo, gate_w):
        del B_x
        B, Sq, M = A_x.shape
        _, Sk, C = A_c_kv.shape
        _, H, D = A_w_q.shape
        _, Hkv, Skb, Dh = B_k_cache.shape
        assert Sq == 1 and Sk == Skb and Dh == 128
        W = min(4096, max(256, Sk // 4))

        any_spec = pl.BlockSpec(memory_space=pl.ANY)
        vmem_spec = pl.BlockSpec(memory_space=pltpu.VMEM)
        n_sems = 64
        kern = functools.partial(_kernel, B=B, H=H, D=D, M=M, C=C, Sk=Sk, Hkv=Hkv,
                                 W=W, KB=KB, mode=mode)
        out = pl.pallas_call(
            kern,
            out_shape=jax.ShapeDtypeStruct((B, M), A_x.dtype),
            in_specs=[vmem_spec, vmem_spec] + [any_spec] * 9,
            out_specs=vmem_spec,
            scratch_shapes=[
                pltpu.VMEM((M * H // 2, D), jnp.uint32),
                pltpu.VMEM((C * H // 2, D), jnp.uint32),
                pltpu.VMEM((C * H // 2, D), jnp.uint32),
                pltpu.VMEM((H * D, M), _BF),
                pltpu.VMEM((M, H * Dh), _BF),
                pltpu.VMEM((H * Dh, M), _BF),
                pltpu.VMEM((B, Sk, C), _BF),
                pltpu.VMEM((B, Hkv, W, Dh), _BF),
                pltpu.VMEM((B, Hkv, W, Dh), _BF),
                pltpu.VMEM((H, B, D), _F32),
                pltpu.VMEM((C // 128, H * B, 128), _F32),
                pltpu.VMEM((H * B, 128), _F32),
                pltpu.VMEM((C // 128, B * H, 128), _F32),
                pltpu.VMEM((B * H, 128), _F32),
                pltpu.VMEM((H, Sk), _F32),
                pltpu.SemaphoreType.DMA((n_sems,)),
            ],
            compiler_params=pltpu.CompilerParams(
                vmem_limit_bytes=120 * 1024 * 1024),
        )(A_x.reshape(B, M), gate_w.reshape(1, M), A_c_kv,
          A_w_q.reshape(M * H, D), A_w_uk.reshape(C * H, D),
          A_w_uv.reshape(C * H, D), A_w_o.reshape(H * D, M),
          B_k_cache, B_v_cache, B_wq, B_wo)
        return out.reshape(B, Sq, M)
    return fn


@jax.jit
def pallas_gated_mix__compressed_kv_cla__sliding_block_cached__decode_kernel(
    A_x: jax.Array,
    A_c_kv: jax.Array,
    A_w_q: jax.Array,
    A_w_uk: jax.Array,
    A_w_uv: jax.Array,
    A_w_o: jax.Array,
    B_x: jax.Array,
    B_k_cache: jax.Array,
    B_v_cache: jax.Array,
    B_wq: jax.Array,
    B_wo: jax.Array,
    gate_w: jax.Array,
):
    return _build()(A_x, A_c_kv, A_w_q, A_w_uk, A_w_uv, A_w_o, B_x, B_k_cache,
                    B_v_cache, B_wq, B_wo, gate_w)
```

```python
import functools

import jax
import jax.numpy as jnp
import jax.experimental.pallas as pl
import jax.experimental.pallas.tpu as pltpu

_BF = jnp.bfloat16
_F32 = jnp.float32
_NT = (((1,), (1,)), ((), ()))

_KEY_BLOCK = 512
_NUM_SEMS = 4


def _dot(a, b):
    return jnp.dot(a, b, preferred_element_type=_F32)


def _dot_nt(a, b):
    return jax.lax.dot_general(a, b, _NT, preferred_element_type=_F32)


def _spans(splits):
    return list(zip(splits[:-1], splits[1:]))


def _repack(src_bf16, dst_u32, rows_per_step=1024):
    @pl.loop(0, src_bf16.shape[0] // rows_per_step)
    def _(i):
        r = pl.multiple_of(i * rows_per_step, rows_per_step)
        r2 = pl.multiple_of(i * (rows_per_step // 2), rows_per_step // 2)
        dst_u32[pl.ds(r2, rows_per_step // 2), :] = pltpu.bitcast(
            src_bf16[pl.ds(r, rows_per_step), :], jnp.uint32)


def _head_pair(w32, hp, n_rows, n_pairs):
    v = w32[pl.ds(hp, n_rows, stride=n_pairs), :]
    lo = jax.lax.bitcast_convert_type(v << 16, _F32)
    hi = jax.lax.bitcast_convert_type(v & jnp.uint32(0xFFFF0000), _F32)
    return lo.astype(_BF), hi.astype(_BF)


def _kernel(x_hbm, gw_hbm, ckv_hbm, wq_hbm, wuk_hbm, wuv_hbm, wo_hbm, kc_hbm,
            vc_hbm, bq_hbm, bo_hbm, out_ref,
            s_x, s_gw, s_wq, s_wuk, s_wuv, s_wo, s_bq, s_bo, s_ckv, s_k, s_v,
            s_w32, s_q, s_qa, s_sc, s_cx, s_qb, s_p, s_ob, sems,
            *, B, H, D, M, C, Sk, Hkv, W):
    scale_a = float(D) ** -0.5
    scale_b = float(128) ** -0.5
    HP = H // 2
    rep = H // Hkv
    KB = _KEY_BLOCK

    b_splits = (0, B // 2, B)
    bo_splits = (0, 3 * H // 4, 7 * H // 8, H - 1, H)

    groups = []

    def group(name, *pairs):
        groups.append((name, pairs))

    group("wq", (wq_hbm, s_wq), (x_hbm, s_x), (gw_hbm, s_gw))
    group("wuk+bq", (wuk_hbm, s_wuk), (bq_hbm, s_bq))
    for a, b in _spans(b_splits):
        group(("ckv", a),
              (ckv_hbm.at[pl.ds(a, b - a)], s_ckv.at[pl.ds(a, b - a)]))
    group("wuv+wo+k", (wuv_hbm, s_wuv), (wo_hbm, s_wo),
          (kc_hbm.at[:, :, pl.ds(Sk - W, W), :], s_k))
    for a, b in _spans(b_splits):
        group(("v", a),
              (vc_hbm.at[pl.ds(a, b - a), :, pl.ds(Sk - W, W), :],
               s_v.at[pl.ds(a, b - a)]))
    for a, b in _spans(bo_splits):
        group(("bo", a),
              (bo_hbm.at[pl.ds(a * 128, (b - a) * 128)],
               s_bo.at[pl.ds(a * 128, (b - a) * 128)]))

    index = {name: i for i, (name, _) in enumerate(groups)}
    copies = [[pltpu.make_async_copy(s, d, sems.at[i % _NUM_SEMS])
               for s, d in pairs]
              for i, (_, pairs) in enumerate(groups)]
    waited = [0]

    def start(i):
        if i < len(groups):
            for c in copies[i]:
                c.start()

    def wait(name):
        i = index[name]
        assert i == waited[0], (name, i, waited[0])
        waited[0] = i + 1
        for c in copies[i]:
            c.wait()
        start(i + _NUM_SEMS)

    for i in range(_NUM_SEMS):
        start(i)

    wait("wq")
    xb = s_x[...]
    _repack(s_wq, s_w32)

    @pl.loop(0, HP)
    def _(hp):
        w0, w1 = _head_pair(s_w32, hp, M, HP)
        s_q[2 * hp] = _dot(xb, w0)
        s_q[2 * hp + 1] = _dot(xb, w1)

    wait("wuk+bq")
    _repack(s_wuk, s_w32)

    @pl.loop(0, HP)
    def _(hp):
        w0, w1 = _head_pair(s_w32, hp, C, HP)
        for j, w in enumerate((w0, w1)):
            h = 2 * hp + j
            qa = _dot_nt(s_q[h].astype(_BF), w) * scale_a
            for ct in range(C // 128):
                s_qa[ct, pl.ds(pl.multiple_of(h * B, B), B), :] = (
                    qa[:, ct * 128:(ct + 1) * 128])

    qb_all = _dot(xb, s_bq[...]) * scale_b
    for h in range(H):
        s_qb[h * B:(h + 1) * B, :] = qb_all[:, h * 128:(h + 1) * 128]

    def mla_batch(b):
        q = jnp.concatenate(
            [s_qa[ct, pl.ds(b, H, stride=B), :] for ct in range(C // 128)],
            axis=1).astype(_BF)
        m = jnp.full((H, KB), -jnp.inf, _F32)
        for kb in range(Sk // KB):
            s = _dot_nt(q, s_ckv[b, kb * KB:(kb + 1) * KB, :])
            s_sc[:, kb * KB:(kb + 1) * KB] = s
            m = jnp.maximum(m, s)
        m = jnp.max(m, axis=1, keepdims=True)
        l = jnp.zeros((H, KB), _F32)
        acc = jnp.zeros((H, C), _F32)
        for kb in range(Sk // KB):
            p = jnp.exp(s_sc[:, kb * KB:(kb + 1) * KB] - m)
            acc = acc + _dot(p.astype(_BF), s_ckv[b, kb * KB:(kb + 1) * KB, :])
            l = l + p
        cx = acc / jnp.sum(l, axis=1, keepdims=True)
        for ct in range(C // 128):
            s_cx[ct, pl.ds(pl.multiple_of(b * H, H), H), :] = (
                cx[:, ct * 128:(ct + 1) * 128])

    for a, b in _spans(b_splits):
        wait(("ckv", a))
        pl.loop(a, b)(mla_batch)

    wait("wuv+wo+k")
    _repack(s_wuv, s_w32)

    def proj_a(hp, acc):
        w0, w1 = _head_pair(s_w32, hp, C, HP)
        for j, w in enumerate((w0, w1)):
            h = 2 * hp + j
            cxh = jnp.concatenate(
                [s_cx[ct, pl.ds(h, B, stride=H), :] for ct in range(C // 128)],
                axis=1).astype(_BF)
            ctx = _dot(cxh, w).astype(_BF)
            acc = acc + _dot(ctx, s_wo[pl.ds(pl.multiple_of(h * D, D), D), :])
        return acc

    out_a = jax.lax.fori_loop(0, HP, proj_a, jnp.zeros((B, M), _F32))

    gw = s_gw[...].astype(_F32).reshape(1, M)
    g = jax.nn.sigmoid(
        jnp.sum(xb.astype(_F32) * gw, axis=1, keepdims=True))
    out_a = g * out_a

    G = 16 // rep

    @pl.loop(0, B)
    def _(b):
        grp = jax.lax.broadcasted_iota(jnp.int32, (16, W), 0) // rep
        qb = s_qb[pl.ds(b, H, stride=B), :].astype(_BF)
        for j in range(H // 16):
            q16 = qb[16 * j:16 * (j + 1)]
            s = None
            for i in range(G):
                si = _dot_nt(q16, s_k[b, G * j + i])
                s = si if s is None else jnp.where(grp == i, si, s)
            m = jnp.max(s, axis=1, keepdims=True)
            p = jnp.exp(s - m)
            l = jnp.sum(p, axis=1, keepdims=True)
            s_p[b, 16 * j:16 * (j + 1), :] = (p / l).astype(_BF)

    def pv_batch(b):
        grp = jax.lax.broadcasted_iota(jnp.int32, (16, 128), 0) // rep
        for j in range(H // 16):
            p = s_p[b, 16 * j:16 * (j + 1), :]
            o = None
            for i in range(G):
                oi = _dot(p, s_v[b, G * j + i])
                o = oi if o is None else jnp.where(grp == i, oi, o)
            s_ob[pl.ds(pl.multiple_of(b * H + 16 * j, 16), 16), :] = o

    for a, b in _spans(b_splits):
        wait(("v", a))
        pl.loop(a, b)(pv_batch)

    out_b = jnp.zeros((B, M), _F32)
    for a, b in _spans(bo_splits):
        ohs = [s_ob[pl.ds(h, B, stride=H), :].astype(_BF)
               for h in range(a, b)]
        wait(("bo", a))
        for h, oh in zip(range(a, b), ohs):
            out_b = out_b + _dot(oh, s_bo[h * 128:(h + 1) * 128, :])

    assert waited[0] == len(groups)
    out_ref[...] = (out_a + (1.0 - g) * out_b).astype(out_ref.dtype)


@jax.jit
def pallas_gated_mix__compressed_kv_cla__sliding_block_cached__decode_kernel(
    A_x: jax.Array,
    A_c_kv: jax.Array,
    A_w_q: jax.Array,
    A_w_uk: jax.Array,
    A_w_uv: jax.Array,
    A_w_o: jax.Array,
    B_x: jax.Array,
    B_k_cache: jax.Array,
    B_v_cache: jax.Array,
    B_wq: jax.Array,
    B_wo: jax.Array,
    gate_w: jax.Array,
):
    del B_x
    B, Sq, M = A_x.shape
    _, Sk, C = A_c_kv.shape
    _, H, D = A_w_q.shape
    _, Hkv, Skb, Dh = B_k_cache.shape
    assert Sq == 1 and Sk == Skb and D == 128 and Dh == 128
    W = min(4096, max(256, Sk // 4))

    f32, u32 = jnp.float32, jnp.uint32
    out = pl.pallas_call(
        functools.partial(_kernel, B=B, H=H, D=D, M=M, C=C, Sk=Sk, Hkv=Hkv, W=W),
        out_shape=jax.ShapeDtypeStruct((B, M), A_x.dtype),
        in_specs=[pl.BlockSpec(memory_space=pl.ANY)] * 11,
        out_specs=pl.BlockSpec(memory_space=pltpu.VMEM),
        scratch_shapes=[
            pltpu.VMEM((B, M), _BF),
            pltpu.VMEM((M,), _BF),
            pltpu.VMEM((M * H, D), _BF),
            pltpu.VMEM((C * H, D), _BF),
            pltpu.VMEM((C * H, D), _BF),
            pltpu.VMEM((H * D, M), _BF),
            pltpu.VMEM((M, H * Dh), _BF),
            pltpu.VMEM((H * Dh, M), _BF),
            pltpu.VMEM((B, Sk, C), _BF),
            pltpu.VMEM((B, Hkv, W, Dh), _BF),
            pltpu.VMEM((B, Hkv, W, Dh), _BF),
            pltpu.VMEM((max(M, C) * H // 2, D), u32),
            pltpu.VMEM((H, B, D), f32),
            pltpu.VMEM((C // 128, H * B, 128), f32),
            pltpu.VMEM((H, Sk), f32),
            pltpu.VMEM((C // 128, B * H, 128), f32),
            pltpu.VMEM((H * B, 128), f32),
            pltpu.VMEM((B, H, W), _BF),
            pltpu.VMEM((B * H, 128), f32),
            pltpu.SemaphoreType.DMA((_NUM_SEMS,)),
        ],
        compiler_params=pltpu.CompilerParams(
            vmem_limit_bytes=120 * 1024 * 1024),
    )(A_x.reshape(B, M), gate_w, A_c_kv,
      A_w_q.reshape(M * H, D), A_w_uk.reshape(C * H, D),
      A_w_uv.reshape(C * H, D), A_w_o.reshape(H * D, M),
      B_k_cache, B_v_cache, B_wq, B_wo)
    return out.reshape(B, Sq, M)
```
